```python
import os as _os
_os.environ.setdefault('JAX_PLATFORMS', 'cpu')
import jax
import jax.numpy as jnp

def _softmax(x, axis=-1):
    return jax.nn.softmax(x, axis=axis)

def _gelu(x):
    return jax.nn.gelu(x, approximate=True)

def _silu(x):
    return jax.nn.silu(x)

def _sigmoid(x):
    return jax.nn.sigmoid(x)

def _layernorm(x, axis=-1, eps=1e-05):
    m = jnp.mean(x, axis=axis, keepdims=True)
    v = jnp.var(x, axis=axis, keepdims=True)
    return (x - m) / jnp.sqrt(v + eps)

def _scatter_add(tgt, idx, src, axis=0):
    return tgt.at[idx].add(src)

def _segment_sum(src, seg, n):
    return jax.ops.segment_sum(src, seg, n)

class _Rng:

    def __init__(self, key):
        self._k = key

    def _next(self):
        self._k, sub = jax.random.split(self._k)
        return sub

    def normal(self, shape):
        return jax.random.normal(self._next(), shape, dtype=jnp.bfloat16)

    def randint(self, lo, hi, shape):
        return jax.random.randint(self._next(), shape, lo, hi, dtype=jnp.int32)

    def uniform(self, shape, lo=0.0, hi=1.0):
        return jax.random.uniform(self._next(), shape, jnp.bfloat16, lo, hi)

    def permutation(self, n):
        return jax.random.permutation(self._next(), n)
kernel_name = 'parallel_sum__memory_aug_recurrent_mem_tr__dense_activation_gelu__prompt'

def setup_inputs():
    _rng = _Rng(jax.random.key(int.from_bytes(__import__("os").urandom(4), "little")))
    _w = lambda a: (lambda t: t.astype(jnp.bfloat16) if jnp.issubdtype(t.dtype, jnp.floating) else t)(jnp.asarray(a))

    def _A_setup():
        B, S, Dm = (1, 2048, 1024)
        H, Dh = (32, 128)
        M, seg = (8, 32)
        seg = min(seg, S)
        S = S // seg * seg
        return {'x': _w((lambda *s: _rng.normal(s) * 0.05)(B, S, Dm)), 'mem0': _w((lambda *s: _rng.normal(s) * 0.2)(B, M, Dm)), 'Wq': _w((lambda *s: _rng.normal(s) * 0.8)(Dm, H, Dh) * Dm ** (-0.5)), 'Wk': _w((lambda *s: _rng.normal(s) * 0.8)(Dm, H, Dh) * Dm ** (-0.5)), 'Wv': _w((lambda *s: _rng.normal(s) * 0.2)(Dm, H, Dh) * Dm ** (-0.5)), 'Wo': _w((lambda *s: _rng.normal(s) * 0.2)(H, Dh, Dm) * (H * Dh) ** (-0.5)), 'seg_len': seg}
    _A_in = _A_setup()

    def _B_setup():
        B, S, D, F = (1, 2048, 1024, 3584)
        return {'x': _w((lambda *s: _rng.normal(s) * 0.05)(B, S, D)), 'w1': _w((lambda *s: _rng.normal(s) * 0.1)(D, F) * D ** (-0.5)), 'b1': _w((lambda *s: _rng.normal(s) * 0.1)(F) * 0.01), 'w2': _w((lambda *s: _rng.normal(s) * 0.1)(F, D) * F ** (-0.5)), 'b2': _w((lambda *s: _rng.normal(s) * 0.05)(D) * 0.01)}
    _B_in = _B_setup()
    return {'A_x': _A_in['x'], 'A_mem0': _A_in['mem0'], 'A_Wq': _A_in['Wq'], 'A_Wk': _A_in['Wk'], 'A_Wv': _A_in['Wv'], 'A_Wo': _A_in['Wo'], 'A_seg_len': _A_in['seg_len'], 'B_x': _B_in['x'], 'B_w1': _B_in['w1'], 'B_b1': _B_in['b1'], 'B_w2': _B_in['w2'], 'B_b2': _B_in['b2']}

def reference(A_x, A_mem0, A_Wq, A_Wk, A_Wv, A_Wo, A_seg_len, B_x, B_w1, B_b1, B_w2, B_b2):

    def _A_ref(x, mem0, Wq, Wk, Wv, Wo, seg_len):
        B, S, Dm = x.shape
        H, Dh = (Wq.shape[1], Wq.shape[2])
        M = mem0.shape[1]
        scale = Dh ** (-0.5)
        n_seg = S // seg_len
        L = M + seg_len
        idx = jnp.arange(L)
        mask = (idx[:, None] < M) | (idx[:, None] >= idx[None, :])
        mem = mem0
        outs = []
        for s in range(n_seg):
            xs = x[:, s * seg_len:(s + 1) * seg_len, :].copy()
            h = jnp.concatenate([mem, xs], axis=1)
            q = jnp.einsum('btd,dhe->bhte', h, Wq)
            k = jnp.einsum('btd,dhe->bhte', h, Wk)
            v = jnp.einsum('btd,dhe->bhte', h, Wv)
            scores = jnp.einsum('bhqe,bhke->bhqk', q, k) * scale
            scores = jnp.where(mask[None, None], scores, -1000000000.0)
            p = _softmax(scores, axis=-1)
            o = jnp.einsum('bhqk,bhke->bhqe', p, v)
            o = jnp.einsum('bhte,hed->btd', o, Wo)
            mem = o[:, :M, :].copy()
            outs.append(o[:, M:, :])
        return jnp.concatenate(outs, axis=1)

    def _B_ref(x, w1, b1, w2, b2):
        h = jnp.einsum('bsd,df->bsf', x, w1) + b1
        h = _gelu(h)
        return jnp.einsum('bsf,fd->bsd', h, w2) + b2
    x = A_x
    xn = _layernorm(x, axis=-1)
    return x + _A_ref(xn, A_mem0, A_Wq, A_Wk, A_Wv, A_Wo, A_seg_len) + _B_ref(xn, B_w1, B_b1, B_w2, B_b2)
```

```python
import functools
import os
import jax
import jax.numpy as jnp
import numpy as np
from jax.experimental import pallas as pl
from jax.experimental.pallas import tpu as pltpu

f32, bf16, u32 = jnp.float32, jnp.bfloat16, jnp.uint32

S, D, H, DH, M, SEG, F = 2048, 1024, 32, 128, 8, 32, 3584
L = M + SEG
NSEG = S // SEG
FT = F // 128
FA = 14
FB = FT - FA
RB = 256
NRB = S // RB
HG = 4
G = H // HG
KT = D // 128


def _gelu(x):
    c = 0.7978845608028654
    return 0.5 * x * (1.0 + jnp.tanh(c * (x + 0.044715 * (x * x * x))))


def _wt(ref, idxs, rows=None):
    if rows is None:
        ts = [pltpu.bitcast(ref[i], bf16) for i in idxs]
    else:
        ts = [pltpu.bitcast(ref[i, rows, :], bf16) for i in idxs]
    return ts[0] if len(ts) == 1 else jnp.concatenate(ts, axis=1)


def _kernel(x_hbm, mem_hbm, wq_hbm, wk_hbm, wv_hbm, wo_hbm, w1_hbm, b1_hbm, w2_hbm, b2_hbm,
            out_hbm,
            xbuf, xn, acc, outbuf, stage, wqkv, wo, w1, w2, b1v, b2v, membuf, mbuf, hbuf,
            sem_small, sem_x, sem_w1a, sem_w2a, sem_st, sem_late, sem_out):
    def cp_x(i):
        return pltpu.make_async_copy(x_hbm.at[pl.ds(i * RB, RB)], xbuf.at[pl.ds(i * RB, RB)], sem_x.at[i])

    def cp_w1(t, sem):
        return pltpu.make_async_copy(w1_hbm.at[:, pl.ds(t * 128, 128)], w1.at[t].bitcast(bf16), sem)

    def cp_w2(c, half, sem):
        r0, n = (0, FA * 128) if half == 0 else (FA * 128, FB * 128)
        return pltpu.make_async_copy(w2_hbm.at[pl.ds(r0, n), pl.ds(c * 128, 128)],
                                     w2.at[c, pl.ds(r0 // 2, n // 2)].bitcast(bf16), sem)

    def cp_wo(c, sem):
        return pltpu.make_async_copy(wo_hbm.at[:, pl.ds(c * 128, 128)], wo.at[c].bitcast(bf16), sem)

    w_hbms = (wq_hbm, wk_hbm, wv_hbm)
    CH = 16384

    def cp_st(j):
        return pltpu.make_async_copy(w_hbms[j // 2].at[pl.ds((j % 2) * CH, CH)],
                                     stage.at[j].bitcast(bf16), sem_st.at[j])

    small = [pltpu.make_async_copy(b1_hbm, b1v, sem_small),
             pltpu.make_async_copy(b2_hbm, b2v, sem_small),
             pltpu.make_async_copy(mem_hbm, membuf, sem_small)]
    W1G = [(0, 2), (2, 6), (6, 10), (10, 14)]
    cp_x(0).start()
    for c in small:
        c.start()
    for gi, (t0, t1) in enumerate(W1G):
        for t in range(t0, t1):
            cp_w1(t, sem_w1a.at[gi]).start()
    for c in range(KT):
        cp_w2(c, 0, sem_w2a).start()
    for i in range(1, NRB):
        cp_x(i).start()
    for j in range(6):
        cp_st(j).start()
    for c in range(KT):
        cp_wo(c, sem_late).start()
    for t in range(FA, FT):
        cp_w1(t, sem_late).start()
    for c in range(KT):
        cp_w2(c, 1, sem_late).start()

    for c in small:
        c.wait()
    mbuf[...] = membuf[...].astype(f32)

    def ln_block(r0):
        xb = xbuf[pl.ds(r0, RB), :].astype(f32)
        m = jnp.mean(xb, axis=-1, keepdims=True)
        d = xb - m
        v = jnp.mean(d * d, axis=-1, keepdims=True)
        xnb = d * jax.lax.rsqrt(v + 1e-5)
        xn[pl.ds(r0, RB), :] = xnb
        return xb, xnb

    def ffn_a_block(r0, first):
        xb, xnb = ln_block(r0)
        for gi, (t0, t1) in enumerate(W1G):
            if first:
                for t in range(t0, t1):
                    cp_w1(t, sem_w1a.at[gi]).wait()
            for t in range(t0, t1, 2):
                u = jnp.dot(xnb, _wt(w1, range(t, t + 2)), preferred_element_type=f32)
                u = u + b1v[pl.ds(t * 128, 256)].astype(f32)[None, :]
                hbuf[:, pl.ds(t * 128, 256)] = _gelu(u)
        if first:
            for c in range(KT):
                cp_w2(c, 0, sem_w2a).wait()
        hb = hbuf[...]
        for c in range(KT):
            r = jnp.dot(hb, _wt(w2, [c], pl.ds(0, FA * 64)), preferred_element_type=f32)
            cs = pl.ds(c * 128, 128)
            acc[pl.ds(r0, RB), cs] = r + (xbuf[pl.ds(r0, RB), cs].astype(f32) + b2v[cs].astype(f32)[None, :])

    def relayout(j):
        mtx = j // 2
        half = j % 2
        for rr in range(4):
            for p in range(16):
                a = stage[j, pl.ds(2048 * rr + p, 128, stride=16), :]
                lo = pltpu.bitcast(a << 16, f32).astype(bf16)
                hi = pltpu.bitcast(a & jnp.uint32(0xFFFF0000), f32).astype(bf16)
                rows = pl.ds(pl.multiple_of(half * 256 + rr * 64, 64), 64)
                wqkv[mtx * H + 2 * p, rows, :] = pltpu.bitcast(lo, u32)
                wqkv[mtx * H + 2 * p + 1, rows, :] = pltpu.bitcast(hi, u32)

    cp_x(0).wait()
    ffn_a_block(0, True)
    cp_x(1).wait()
    ffn_a_block(RB, False)

    def pro_body(j, c):
        r0 = pl.multiple_of((j + 2) * RB, RB)
        cp_x_dyn = pltpu.make_async_copy(x_hbm.at[pl.ds(r0, RB)], xbuf.at[pl.ds(r0, RB)], sem_x.at[j + 2])
        cp_x_dyn.wait()
        pltpu.make_async_copy(wq_hbm.at[pl.ds(0, CH)], stage.at[j].bitcast(bf16), sem_st.at[j]).wait()
        relayout(j)
        ffn_a_block(r0, False)
        return c
    jax.lax.fori_loop(0, NRB - 2, pro_body, 0)

    for c in range(KT):
        cp_wo(c, sem_late).wait()
    for t in range(FA, FT):
        cp_w1(t, sem_late).wait()
    for c in range(KT):
        cp_w2(c, 1, sem_late).wait()

    scale = DH ** -0.5

    def cp_out(r0):
        return pltpu.make_async_copy(outbuf.at[pl.ds(r0, SEG)], out_hbm.at[pl.ds(r0, SEG)], sem_out)

    def step(s, carry):
        ii = jax.lax.broadcasted_iota(jnp.int32, (L, L), 0)
        jj = jax.lax.broadcasted_iota(jnp.int32, (L, L), 1)
        mask = (ii < M) | (ii >= jj)
        r0 = pl.multiple_of(s * SEG, SEG)
        xs = xn[pl.ds(r0, SEG), :]
        h = jnp.concatenate([mbuf[...], xs], axis=0)
        q, kk, v, e, rl, o, ff = {}, {}, {}, {}, {}, {}, {}
        st = dict(acc=None, facc=None)
        hs = lambda g, m: range(m * H + g * HG, m * H + (g + 1) * HG)

        def Q(g):
            q[g] = jnp.dot(h, _wt(wqkv, hs(g, 0)), preferred_element_type=f32)

        def K(g):
            kk[g] = jnp.dot(h, _wt(wqkv, hs(g, 1)), preferred_element_type=f32).astype(bf16)

        def V(g):
            v[g] = jnp.dot(h, _wt(wqkv, hs(g, 2)), preferred_element_type=f32).astype(bf16)

        def Sc(g):
            es, rls = [], []
            for j in range(HG):
                sl = slice(j * 128, (j + 1) * 128)
                sc = jax.lax.dot_general(q[g][:, sl], kk[g][:, sl], (((1,), (1,)), ((), ())),
                                         preferred_element_type=f32) * scale
                sc = jnp.where(mask, sc, -1e9)
                mx = jnp.max(sc, axis=-1, keepdims=True)
                ex = jnp.exp(sc - mx)
                es.append(ex)
                rls.append(1.0 / jnp.sum(ex, axis=-1, keepdims=True))
            e[g] = es
            rl[g] = rls

        def PV(g):
            os_ = []
            for j in range(HG):
                sl = slice(j * 128, (j + 1) * 128)
                os_.append(jnp.dot(e[g][j], v[g][:, sl], preferred_element_type=f32) * rl[g][j])
            o[g] = jnp.concatenate(os_, axis=1)

        def WO(g):
            r = jnp.dot(o[g], _wt(wo, range(KT), pl.ds(g * HG * 64, HG * 64)), preferred_element_type=f32)
            st["acc"] = r if st["acc"] is None else st["acc"] + r

        def UP(i, t0, t1):
            u = jnp.dot(xs, _wt(w1, range(t0, t1)), preferred_element_type=f32)
            u = u + b1v[pl.ds(t0 * 128, (t1 - t0) * 128)].astype(f32)[None, :]
            ff[i] = _gelu(u)

        def DN(i, t0, t1):
            r = jnp.dot(ff[i], _wt(w2, range(KT), pl.ds(t0 * 64, (t1 - t0) * 64)), preferred_element_type=f32)
            st["facc"] = r if st["facc"] is None else st["facc"] + r

        hf = FA + 8
        Q(0); K(0); V(0)
        for g in range(G):
            if g + 1 < G:
                Q(g + 1)
            else:
                UP(0, FA, hf)
            Sc(g)
            if g + 1 < G:
                K(g + 1)
            else:
                UP(1, hf, FT)
            if g >= 1:
                WO(g - 1)
            if g == 0:
                V(1)
            PV(g)
            if g + 1 < G and g > 0:
                V(g + 1)
        DN(0, FA, hf)
        WO(G - 1)
        a = st["acc"]
        mbuf[...] = a[0:M]
        DN(1, hf, FT)
        outbuf[pl.ds(r0, SEG), :] = (acc[pl.ds(r0, SEG), :] + a[M:L] + st["facc"]).astype(bf16)
        cp_out(r0).start()
        return carry

    jax.lax.fori_loop(0, NSEG, step, 0)

    def wait_out(s, c):
        cp_out(pl.multiple_of(s * SEG, SEG)).wait()
        return c
    jax.lax.fori_loop(0, NSEG, wait_out, 0)


@functools.partial(jax.jit, static_argnames=["A_seg_len"])
def pallas_parallel_sum__memory_aug_recurrent_mem_tr__dense_activation_gelu__prompt_kernel(
        A_x, A_mem0, A_Wq, A_Wk, A_Wv, A_Wo, A_seg_len, B_x, B_w1, B_b1, B_w2, B_b2):
    assert A_seg_len == SEG
    any_spec = pl.BlockSpec(memory_space=pl.ANY)
    DMA = pltpu.SemaphoreType.DMA
    out = pl.pallas_call(
        _kernel,
        out_shape=jax.ShapeDtypeStruct((S, D), bf16),
        in_specs=[any_spec] * 10,
        out_specs=any_spec,
        scratch_shapes=[
            pltpu.VMEM((S, D), bf16),
            pltpu.VMEM((S, D), f32),
            pltpu.VMEM((S, D), f32),
            pltpu.VMEM((S, D), bf16),
            pltpu.VMEM((6, 8192, 128), u32),
            pltpu.VMEM((3 * H, D // 2, 128), u32),
            pltpu.VMEM((KT, H * DH // 2, 128), u32),
            pltpu.VMEM((FT, D // 2, 128), u32),
            pltpu.VMEM((KT, F // 2, 128), u32),
            pltpu.VMEM((F,), bf16),
            pltpu.VMEM((D,), bf16),
            pltpu.VMEM((M, D), bf16),
            pltpu.VMEM((M, D), f32),
            pltpu.VMEM((RB, FA * 128), f32),
            DMA(()), DMA((NRB,)), DMA((4,)), DMA(()), DMA((6,)), DMA(()), DMA(()),
        ],
        compiler_params=pltpu.CompilerParams(vmem_limit_bytes=120 * 2**20),
        name="rmt_ffn",
    )(A_x.reshape(S, D), A_mem0.reshape(M, D), A_Wq.reshape(D * H, DH), A_Wk.reshape(D * H, DH),
      A_Wv.reshape(D * H, DH), A_Wo.reshape(H * DH, D), B_w1, B_b1, B_w2, B_b2)
    return out.reshape(1, S, D)
```

```python
import functools
import jax
import jax.numpy as jnp
import numpy as np
from jax.experimental import pallas as pl
from jax.experimental.pallas import tpu as pltpu

f32, bf16, u32 = jnp.float32, jnp.bfloat16, jnp.uint32

S, D, H, DH, M, SEG, F = 2048, 1024, 32, 128, 8, 32, 3584
L = M + SEG
NSEG = S // SEG
FT = F // 128
FA = 14
FB = FT - FA
RB = 256
NRB = S // RB
HG = 4
G = H // HG
KT = D // 128
TIE_RL = 0
TIE_UP = 1
TIE_LN = 1
UNROLL = 2
NSTEPS = NSEG


def _gelu(x):
    c = 0.7978845608028654
    return 0.5 * x * (1.0 + jnp.tanh(c * (x + 0.044715 * (x * x * x))))


def _wt(ref, idxs, rows=None):
    if rows is None:
        ts = [pltpu.bitcast(ref[i], bf16) for i in idxs]
    else:
        ts = [pltpu.bitcast(ref[i, rows, :], bf16) for i in idxs]
    return ts[0] if len(ts) == 1 else jnp.concatenate(ts, axis=1)


def _kernel(x_hbm, mem_hbm, wq_hbm, wk_hbm, wv_hbm, wo_hbm, w1_hbm, b1_hbm, w2_hbm, b2_hbm,
            out_hbm,
            xbuf, xn, acc, outbuf, stage, wqkv, wo, w1, w2, b1v, b2v, b1f, b2f, membuf, mbuf, hbuf,
            sem_small, sem_x, sem_w1a, sem_w2a, sem_st, sem_late, sem_out):
    def mo(v, k):
        return v if isinstance(v, int) else pl.multiple_of(v, k)

    def cp_x(i):
        rows = pl.ds(mo(i * RB, RB), RB)
        return pltpu.make_async_copy(x_hbm.at[rows], xbuf.at[rows], sem_x.at[i])

    def cp_w1(t, sem):
        return pltpu.make_async_copy(w1_hbm.at[:, pl.ds(mo(t * 128, 128), 128)], w1.at[t].bitcast(bf16), sem)

    def cp_w2(c, half, sem):
        r0, n = (0, FA * 128) if half == 0 else (FA * 128, FB * 128)
        return pltpu.make_async_copy(w2_hbm.at[pl.ds(r0, n), pl.ds(mo(c * 128, 128), 128)],
                                     w2.at[c, pl.ds(r0 // 2, n // 2)].bitcast(bf16), sem)

    def cp_wo(c, sem):
        return pltpu.make_async_copy(wo_hbm.at[:, pl.ds(mo(c * 128, 128), 128)], wo.at[c].bitcast(bf16), sem)

    w_hbms = (wq_hbm, wk_hbm, wv_hbm)

    def cp_st(mi, p, sem):
        return pltpu.make_async_copy(w_hbms[mi].bitcast(u32).at[:, p, :], stage.at[mi * 16 + p], sem)

    small = [pltpu.make_async_copy(b1_hbm, b1v, sem_small),
             pltpu.make_async_copy(b2_hbm, b2v, sem_small),
             pltpu.make_async_copy(mem_hbm, membuf, sem_small)]
    def issue_loop(n, fn):
        def body(i, c):
            fn(i)
            return c
        jax.lax.fori_loop(0, n, body, 0)

    cp_x(0).start()
    cp_x(1).start()
    for c in small:
        c.start()
    issue_loop(FA, lambda t: cp_w1(t, sem_w1a.at[t]).start())
    issue_loop(KT, lambda c: cp_w2(c, 0, sem_w2a).start())
    for i in range(2, NRB):
        cp_x(i).start()
    def issue_stage(mi):
        for p in range(16):
            cp_st(mi, p, sem_st.at[2 * mi + p // 8]).start()

    def issue_late():
        for c in range(KT):
            cp_wo(c, sem_late).start()
        for t in range(FA, FT):
            cp_w1(t, sem_late).start()
        for c in range(KT):
            cp_w2(c, 1, sem_late).start()


    for c in small:
        c.wait()
    mbuf[...] = membuf[...].astype(f32)
    for t in range(FT):
        b1f[t] = jnp.broadcast_to(b1v[pl.ds(t * 128, 128)].astype(f32)[None, :], (8, 128))
    for c in range(KT):
        b2f[c] = jnp.broadcast_to(b2v[pl.ds(c * 128, 128)].astype(f32)[None, :], (8, 128))

    def ln_rows(r0, n):
        xb = xbuf[pl.ds(r0, n), :].astype(f32)
        m = jnp.mean(xb, axis=-1, keepdims=True)
        d = xb - m
        v = jnp.mean(d * d, axis=-1, keepdims=True)
        xn[pl.ds(r0, n), :] = d * jax.lax.rsqrt(v + 1e-5)

    def relayout_unit(u, d0, nd):
        a = stage[u, pl.ds(d0, nd), :]
        rows = pl.ds(d0 // 2, nd // 2)
        wqkv[2 * u, rows, :] = pltpu.bitcast(a.astype(jnp.uint16), u32)
        wqkv[2 * u + 1, rows, :] = pltpu.bitcast((a >> 16).astype(jnp.uint16), u32)

    def up_dot(r0, hr0, t, tie=None):
        u = jnp.dot(xn[pl.ds(r0, RB), :], _wt(w1, (t, t + 1)), preferred_element_type=f32)
        bias = jnp.concatenate([b1f[t], b1f[t + 1]], axis=1)
        if tie is not None:
            bias = tie(bias)
        u = (u.reshape(RB // 8, 8, 256) + bias[None]).reshape(RB, 256)
        g = _gelu(u)
        hbuf[pl.ds(hr0, RB), pl.ds(mo(t * 128, 128), 256)] = g
        return g[0:8, 0:128]

    def dn_dot(r0, hr0, c, tie=None):
        r = jnp.dot(hbuf[pl.ds(hr0, RB), :], _wt(w2, [c], pl.ds(0, FA * 64)), preferred_element_type=f32)
        cs = pl.ds(mo(c * 128, 128), 128)
        bias = b2f[c]
        if tie is not None:
            bias = tie(bias)
        xb = xbuf[pl.ds(r0, RB), cs].astype(f32)
        xb = (xb.reshape(RB // 8, 8, 128) + bias[None]).reshape(RB, 128)
        acc[pl.ds(r0, RB), cs] = r + xb
        return r[0:8, :]

    cp_x(0).wait()
    cp_x(1).wait()
    issue_stage(0)
    ln_rows(0, RB)
    ln_rows(RB, RB)
    def upA(i, c):
        t = i * 2
        cp_w1(t, sem_w1a.at[t]).wait()
        cp_w1(t + 1, sem_w1a.at[t + 1]).wait()
        up_dot(0, 0, t)
        up_dot(RB, RB, t)
        return c
    jax.lax.fori_loop(0, FA // 2, upA, 0)
    for c in range(KT):
        cp_w2(c, 0, sem_w2a).wait()
    cp_x(2).wait()
    issue_stage(1)
    issue_stage(2)
    n = RB // 4

    def dnA(i, carry):
        c = i * 2
        dn_dot(0, 0, c)
        dn_dot(RB, RB, c)
        ln_rows(pl.multiple_of(2 * RB + i * n, n), n)
        dn_dot(0, 0, c + 1)
        dn_dot(RB, RB, c + 1)
        return carry
    jax.lax.fori_loop(0, KT // 2, dnA, 0)

    for i in range(3, NRB):
        cp_x(i).wait()
    NDOT = FA // 2 + KT
    RLD = 256
    units = [(i, d0) for i in range(8) for d0 in range(0, D, RLD)]

    def pro_body(j, carry):
        r0 = pl.multiple_of((j + 2) * RB, RB)
        rn = pl.multiple_of(jnp.minimum(j + 3, NRB - 1) * RB, RB)
        for p in range(8):
            cp_st(0, p, sem_st.at[j]).wait()

        @pl.when(j == 1)
        def _():
            issue_late()
        pred = j < 1000
        ln_dummy_row = pl.multiple_of(jnp.minimum(rn, S - 8), 8)
        ud = jnp.minimum(j, 5) * 8

        def rl_group(i, prev):
            lo, hi = (i * len(units)) // (NDOT - 1), ((i + 1) * len(units)) // (NDOT - 1)
            for (ui, d0) in units[lo:hi]:
                relayout_unit(j * 8 + ui, d0, RLD)
            (ui, d0) = units[hi - 1]
            d = wqkv[2 * (ud + ui) + 1, pl.ds((d0 + RLD) // 2 - 8, 8), :]
            return pltpu.bitcast(d, f32)

        def mk_tie(ds):
            def tie(b):
                for d in ds:
                    if d.shape[1] != b.shape[1]:
                        d = jnp.concatenate([d] * (b.shape[1] // d.shape[1]), axis=1)
                    b = jnp.where(pred, b, d)
                return b
            return tie if ds else None

        i = 0
        prev = None
        for t in range(0, FA, 2):
            ds = [rl_group(i - 1, prev)] if i >= 1 else []
            prev = up_dot(r0, 0, t, mk_tie(ds if TIE_RL else []))
            i += 1
        for c in range(KT):
            ds = [rl_group(i - 1, prev)]
            ds = ds if TIE_RL else []
            if c in (1, 3, 5, 7):
                k = c // 2
                ln_rows(pl.multiple_of(rn + k * n, n), n)
                if TIE_LN:
                    ds.append(xn[pl.ds(pl.multiple_of(ln_dummy_row + k * n + n - 8, 8), 8), 0:128])
            prev = dn_dot(r0, 0, c, mk_tie(ds))
            i += 1
        return carry
    jax.lax.fori_loop(0, NRB - 2, pro_body, 0)

    for c in range(KT):
        cp_wo(c, sem_late).wait()
    for t in range(FA, FT):
        cp_w1(t, sem_late).wait()
    for c in range(KT):
        cp_w2(c, 1, sem_late).wait()

    scale = DH ** -0.5

    def cp_out(r0):
        return pltpu.make_async_copy(outbuf.at[pl.ds(r0, SEG)], out_hbm.at[pl.ds(r0, SEG)], sem_out)

    def step(s, mem):
        ii = jax.lax.broadcasted_iota(jnp.int32, (L, L), 0)
        jj = jax.lax.broadcasted_iota(jnp.int32, (L, L), 1)
        mask = (ii < M) | (ii >= jj)
        r0 = pl.multiple_of(s * SEG, SEG)
        xs = xn[pl.ds(r0, SEG), :]
        h = jnp.concatenate([mem, xs], axis=0)
        q, kk, v, e, rl, o, ff = {}, {}, {}, {}, {}, {}, {}
        st = dict(acc=None, facc=None)
        hs = lambda g, m: range(m * H + g * HG, m * H + (g + 1) * HG)

        def Q(g):
            q[g] = jnp.dot(h, _wt(wqkv, hs(g, 0)), preferred_element_type=f32)

        def K(g):
            kk[g] = jnp.dot(h, _wt(wqkv, hs(g, 1)), preferred_element_type=f32).astype(bf16)

        def V(g):
            v[g] = jnp.dot(h, _wt(wqkv, hs(g, 2)), preferred_element_type=f32).astype(bf16)

        def Sc(g):
            es, rls = [], []
            for j in range(HG):
                sl = slice(j * 128, (j + 1) * 128)
                sc = jax.lax.dot_general(q[g][:, sl], kk[g][:, sl], (((1,), (1,)), ((), ())),
                                         preferred_element_type=f32) * scale
                sc = jnp.where(mask, sc, -1e9)
                mx = jnp.max(sc, axis=-1, keepdims=True)
                ex = jnp.exp(sc - mx)
                es.append(ex)
                rls.append(1.0 / jnp.sum(ex, axis=-1, keepdims=True))
            e[g] = es
            rl[g] = rls

        def PV(g):
            os_ = []
            for j in range(HG):
                sl = slice(j * 128, (j + 1) * 128)
                os_.append(jnp.dot(e[g][j], v[g][:, sl], preferred_element_type=f32) * rl[g][j])
            o[g] = jnp.concatenate(os_, axis=1)

        def WO(g):
            r = jnp.dot(o[g], _wt(wo, range(KT), pl.ds(g * HG * 64, HG * 64)), preferred_element_type=f32)
            st["acc"] = r if st["acc"] is None else st["acc"] + r

        def UP(i, t0, t1):
            u = jnp.dot(xs, _wt(w1, range(t0, t1)), preferred_element_type=f32)
            bias = jnp.concatenate([b1f[t] for t in range(t0, t1)], axis=1)
            u = (u.reshape(SEG // 8, 8, (t1 - t0) * 128) + bias[None]).reshape(SEG, (t1 - t0) * 128)
            ff[i] = _gelu(u)

        def DN(i, t0, t1):
            r = jnp.dot(ff[i], _wt(w2, range(KT), pl.ds(t0 * 64, (t1 - t0) * 64)), preferred_element_type=f32)
            st["facc"] = (acc[pl.ds(r0, SEG), :] if st["facc"] is None else st["facc"]) + r

        hf = FA + 8
        Q(0); K(0); V(0)
        for g in range(G):
            if g + 1 < G:
                Q(g + 1)
            else:
                UP(0, FA, hf)
            Sc(g)
            if g + 1 < G:
                K(g + 1)
            else:
                UP(1, hf, FT)
            if g >= 1:
                WO(g - 1)
            if g == 0:
                V(1)
            PV(g)
            if g + 1 < G and g > 0:
                V(g + 1)
        DN(0, FA, hf)
        WO(G - 1)
        a = st["acc"]
        DN(1, hf, FT)
        outbuf[pl.ds(r0, SEG), :] = (a[M:L] + st["facc"]).astype(bf16)
        cp_out(r0).start()
        return a[0:M]

    def steps(i, carry):
        mem = mbuf[...]
        for u in range(UNROLL):
            mem = step(i * UNROLL + u, mem)
        mbuf[...] = mem
        return carry

    jax.lax.fori_loop(0, NSTEPS // UNROLL, steps, 0)

    def wait_out(s, c):
        cp_out(pl.multiple_of(s * SEG, SEG)).wait()
        return c
    jax.lax.fori_loop(0, NSTEPS, wait_out, 0)


@functools.partial(jax.jit, static_argnames=["A_seg_len"])
def pallas_parallel_sum__memory_aug_recurrent_mem_tr__dense_activation_gelu__prompt_kernel(
        A_x, A_mem0, A_Wq, A_Wk, A_Wv, A_Wo, A_seg_len, B_x, B_w1, B_b1, B_w2, B_b2):
    assert A_seg_len == SEG
    any_spec = pl.BlockSpec(memory_space=pl.ANY)
    DMA = pltpu.SemaphoreType.DMA
    out = pl.pallas_call(
        _kernel,
        out_shape=jax.ShapeDtypeStruct((S, D), bf16),
        in_specs=[any_spec] * 10,
        out_specs=any_spec,
        scratch_shapes=[
            pltpu.VMEM((S, D), bf16),
            pltpu.VMEM((S, D), f32),
            pltpu.VMEM((S, D), f32),
            pltpu.VMEM((S, D), bf16),
            pltpu.VMEM((48, D, 128), u32),
            pltpu.VMEM((3 * H, D // 2, 128), u32),
            pltpu.VMEM((KT, H * DH // 2, 128), u32),
            pltpu.VMEM((FT, D // 2, 128), u32),
            pltpu.VMEM((KT, F // 2, 128), u32),
            pltpu.VMEM((F,), bf16),
            pltpu.VMEM((D,), bf16),
            pltpu.VMEM((FT, 8, 128), f32),
            pltpu.VMEM((KT, 8, 128), f32),
            pltpu.VMEM((M, D), bf16),
            pltpu.VMEM((M, D), f32),
            pltpu.VMEM((2 * RB, FA * 128), f32),
            DMA(()), DMA((NRB,)), DMA((FA,)), DMA(()), DMA((6,)), DMA(()), DMA(()),
        ],
        compiler_params=pltpu.CompilerParams(vmem_limit_bytes=120 * 2**20),
        name="rmt_ffn",
    )(A_x.reshape(S, D), A_mem0.reshape(M, D), A_Wq, A_Wk,
      A_Wv, A_Wo.reshape(H * DH, D), B_w1, B_b1, B_w2, B_b2)
    return out.reshape(1, S, D)
```

```python
import functools

import jax
import jax.numpy as jnp
from jax.experimental import pallas as pl
from jax.experimental.pallas import tpu as pltpu

f32, bf16, u32 = jnp.float32, jnp.bfloat16, jnp.uint32

S, D, H, DH, M, SEG, F = 2048, 1024, 32, 128, 8, 32, 3584
L = M + SEG
NSEG = S // SEG
KT = D // 128
FT = F // 128
FA = 14
RB = 256
NRB = S // RB
HG = 4
G = H // HG
NPAIR = 3 * H // 2
UNROLL = 2


def _gelu(x):
    c = 0.7978845608028654
    hx = 0.5 * x
    return hx + hx * jnp.tanh(x * (c + (c * 0.044715) * (x * x)))


def _mult(v, k):
    return v if isinstance(v, int) else pl.multiple_of(v, k)


def _wt(ref, idxs, rows=None):
    ts = [pltpu.bitcast(ref[i] if rows is None else ref[i, rows, :], bf16) for i in idxs]
    return ts[0] if len(ts) == 1 else jnp.concatenate(ts, axis=1)


def _add_rows(a, b8):
    r, n = a.shape
    return (a.reshape(r // 8, 8, n) + b8[None]).reshape(r, n)


def _loop(n, fn):
    def body(i, carry):
        fn(i)
        return carry
    jax.lax.fori_loop(0, n, body, 0)


def _kernel(x_hbm, mem_hbm, wq_hbm, wk_hbm, wv_hbm, wo_hbm, w1_hbm, b1_hbm, w2_hbm, b2_hbm,
            out_hbm,
            xbuf, xn, acc, outbuf, stage, wqkv, wo, w1, w2, b1v, b2v, b1f, b2f, membuf, mbuf, hbuf,
            sem_small, sem_x, sem_w1a, sem_w2a, sem_st, sem_late, sem_out):
    def cp_x(i):
        rows = pl.ds(_mult(i * RB, RB), RB)
        return pltpu.make_async_copy(x_hbm.at[rows], xbuf.at[rows], sem_x.at[i])

    def cp_w1(t, sem):
        cols = pl.ds(_mult(t * 128, 128), 128)
        return pltpu.make_async_copy(w1_hbm.at[:, cols], w1.at[t].bitcast(bf16), sem)

    def cp_w2(c, first, sem):
        r0, n = (0, FA * 128) if first else (FA * 128, (FT - FA) * 128)
        cols = pl.ds(_mult(c * 128, 128), 128)
        return pltpu.make_async_copy(w2_hbm.at[pl.ds(r0, n), cols],
                                     w2.at[c, pl.ds(r0 // 2, n // 2)].bitcast(bf16), sem)

    def cp_wo(c, sem):
        return pltpu.make_async_copy(wo_hbm.at[:, pl.ds(c * 128, 128)], wo.at[c].bitcast(bf16), sem)

    def cp_pair(mi, p):
        u = mi * (H // 2) + p
        src = (wq_hbm, wk_hbm, wv_hbm)[mi].bitcast(u32).at[:, p, :]
        return pltpu.make_async_copy(src, stage.at[u], sem_st.at[u // 8])

    def cp_out(r0):
        rows = pl.ds(r0, SEG)
        return pltpu.make_async_copy(outbuf.at[rows], out_hbm.at[rows], sem_out)

    cp_small = (pltpu.make_async_copy(b1_hbm, b1v, sem_small.at[0]),
                pltpu.make_async_copy(b2_hbm, b2v, sem_small.at[1]),
                pltpu.make_async_copy(mem_hbm, membuf, sem_small.at[2]))

    def ln_rows(r0, n):
        xb = xbuf[pl.ds(r0, n), :].astype(f32)
        d = xb - jnp.mean(xb, axis=-1, keepdims=True)
        var = jnp.mean(d * d, axis=-1, keepdims=True)
        xn[pl.ds(r0, n), :] = d * jax.lax.rsqrt(var + 1e-5)

    def up_dot(r0, hr0, t):
        u = jnp.dot(xn[pl.ds(r0, RB), :], _wt(w1, (t, t + 1)), preferred_element_type=f32)
        u = _add_rows(u, jnp.concatenate([b1f[t], b1f[t + 1]], axis=1))
        hbuf[pl.ds(hr0, RB), pl.ds(_mult(t * 128, 128), 256)] = _gelu(u)

    def dn_dot(r0, hr0, c, tie=None):
        r = jnp.dot(hbuf[pl.ds(hr0, RB), :], _wt(w2, (c,), pl.ds(0, FA * 64)), preferred_element_type=f32)
        cs = pl.ds(_mult(c * 128, 128), 128)
        bias = b2f[c] if tie is None else tie(b2f[c])
        acc[pl.ds(r0, RB), cs] = r + _add_rows(xbuf[pl.ds(r0, RB), cs].astype(f32), bias)

    def repack(u, d0, nd):
        a = stage[u, pl.ds(d0, nd), :]
        rows = pl.ds(d0 // 2, nd // 2)
        wqkv[2 * u, rows, :] = pltpu.bitcast(a.astype(jnp.uint16), u32)
        wqkv[2 * u + 1, rows, :] = pltpu.bitcast((a >> 16).astype(jnp.uint16), u32)

    cp_x(0).start()
    cp_x(1).start()
    for c in cp_small:
        c.start()
    _loop(FA, lambda t: cp_w1(t, sem_w1a.at[t]).start())
    _loop(KT, lambda c: cp_w2(c, True, sem_w2a).start())
    for i in range(2, NRB):
        cp_x(i).start()

    cp_x(0).wait()
    for p in range(H // 2):
        cp_pair(0, p).start()
    ln_rows(0, RB)
    cp_x(1).wait()
    ln_rows(RB, RB)
    cp_small[0].wait()
    for t in range(FT):
        b1f[t] = jnp.broadcast_to(b1v[pl.ds(t * 128, 128)].astype(f32)[None, :], (8, 128))

    for t0, t1 in ((0, 2), (2, 6), (6, FA)):
        for t in range(t0, t1):
            cp_w1(t, sem_w1a.at[t]).wait()
        for t in range(t0, t1, 2):
            up_dot(0, 0, t)
            up_dot(RB, RB, t)

    for c in range(KT):
        cp_w2(c, True, sem_w2a).wait()
    cp_x(2).wait()
    cp_small[1].wait()
    cp_small[2].wait()
    mbuf[...] = membuf[...].astype(f32)
    for c in range(KT):
        b2f[c] = jnp.broadcast_to(b2v[pl.ds(c * 128, 128)].astype(f32)[None, :], (8, 128))
    for mi in (1, 2):
        for p in range(H // 2):
            cp_pair(mi, p).start()

    def dn_first(i):
        n = RB // 4
        for k in range(2):
            c = 2 * (2 * i + k)
            dn_dot(0, 0, c)
            dn_dot(RB, RB, c)
            ln_rows(pl.multiple_of(2 * RB + (2 * i + k) * n, n), n)
            dn_dot(0, 0, c + 1)
            dn_dot(RB, RB, c + 1)
    _loop(2, dn_first)

    for i in range(3, NRB):
        cp_x(i).wait()
    ndot = FA // 2 + KT
    pieces = [(u, d0) for u in range(8) for d0 in range(0, D, 128)]

    def ffn_block(j):
        r0 = pl.multiple_of((j + 2) * RB, RB)
        rn = pl.multiple_of(jnp.minimum(j + 3, NRB - 1) * RB, RB)
        chunk = stage.at[pl.ds(j * 8, 8)]
        pltpu.make_async_copy(chunk, chunk, sem_st.at[j]).wait()

        @pl.when(j == 1)
        def _():
            for c in range(KT):
                cp_wo(c, sem_late).start()
            for t in range(FA, FT):
                cp_w1(t, sem_late).start()
            for c in range(KT):
                cp_w2(c, False, sem_late).start()

        def repack_part(i):
            for u, d0 in pieces[i * len(pieces) // (ndot - 1):(i + 1) * len(pieces) // (ndot - 1)]:
                repack(j * 8 + u, d0, 128)

        for i, t in enumerate(range(0, FA, 2)):
            if i >= 1:
                repack_part(i - 1)
            up_dot(r0, 0, t)
        live = j < NRB
        n = RB // KT
        for c in range(KT):
            repack_part(FA // 2 + c - 1)
            for r in range(0, n, 8):
                ln_rows(pl.multiple_of(rn + c * n + r, 8), 8)
            done = xn[pl.ds(pl.multiple_of(rn + (c + 1) * n - 8, 8), 8), 0:128]
            dn_dot(r0, 0, c, lambda b, done=done: jnp.where(live, b, done))
    _loop(NRB - 2, ffn_block)

    for c in range(KT):
        cp_wo(c, sem_late).wait()
    for t in range(FA, FT):
        cp_w1(t, sem_late).wait()
    for c in range(KT):
        cp_w2(c, False, sem_late).wait()

    scale = DH ** -0.5

    def step(s, mem):
        ii = jax.lax.broadcasted_iota(jnp.int32, (L, L), 0)
        jj = jax.lax.broadcasted_iota(jnp.int32, (L, L), 1)
        mask = (ii < M) | (ii >= jj)
        r0 = pl.multiple_of(s * SEG, SEG)
        xs = xn[pl.ds(r0, SEG), :]
        h = jnp.concatenate([mem, xs], axis=0)
        q, k, v, e, rl, o, ff = {}, {}, {}, {}, {}, {}, {}
        st = dict(attn=None, ffn=None)
        heads = lambda g, mi: range(mi * H + g * HG, mi * H + (g + 1) * HG)
        lanes = [slice(j * DH, (j + 1) * DH) for j in range(HG)]

        def proj(dst, g, mi):
            dst[g] = jnp.dot(h, _wt(wqkv, heads(g, mi)), preferred_element_type=f32)

        def scores(g):
            e[g], rl[g] = [], []
            for sl in lanes:
                sc = jax.lax.dot_general(q[g][:, sl], k[g][:, sl].astype(bf16), (((1,), (1,)), ((), ())),
                                         preferred_element_type=f32) * scale
                sc = jnp.where(mask, sc, -1e9)
                ex = jnp.exp(sc - jnp.max(sc, axis=-1, keepdims=True))
                tot = jnp.sum(ex, axis=-1, keepdims=True)
                r = pltpu.reciprocal(tot, approx=True)
                e[g].append(ex)
                rl[g].append(r * (2.0 - tot * r))

        def pv(g):
            o[g] = jnp.concatenate(
                [jnp.dot(e[g][j], v[g][:, sl].astype(bf16), preferred_element_type=f32) * rl[g][j]
                 for j, sl in enumerate(lanes)], axis=1)

        def out_proj(g):
            r = jnp.dot(o[g], _wt(wo, range(KT), pl.ds(g * HG * 64, HG * 64)), preferred_element_type=f32)
            st["attn"] = r if st["attn"] is None else st["attn"] + r

        def up(i, t0, t1):
            u = jnp.dot(xs, _wt(w1, range(t0, t1)), preferred_element_type=f32)
            ff[i] = _gelu(_add_rows(u, jnp.concatenate([b1f[t] for t in range(t0, t1)], axis=1)))

        def down(i, t0, t1):
            r = jnp.dot(ff[i], _wt(w2, range(KT), pl.ds(t0 * 64, (t1 - t0) * 64)), preferred_element_type=f32)
            st["ffn"] = (acc[pl.ds(r0, SEG), :] if st["ffn"] is None else st["ffn"]) + r

        mid = FA + 8
        proj(q, 0, 0)
        proj(k, 0, 1)
        proj(v, 0, 2)
        for g in range(G):
            last = g + 1 == G
            up(0, FA, mid) if last else proj(q, g + 1, 0)
            scores(g)
            up(1, mid, FT) if last else proj(k, g + 1, 1)
            if g == 0:
                proj(v, 1, 2)
            else:
                out_proj(g - 1)
            pv(g)
            if 0 < g < G - 1:
                proj(v, g + 1, 2)
        down(0, FA, mid)
        out_proj(G - 1)
        attn = st["attn"]
        down(1, mid, FT)
        outbuf[pl.ds(r0, SEG), :] = (attn[M:L] + st["ffn"]).astype(bf16)
        cp_out(r0).start()
        return attn[0:M]

    def steps(i):
        mem = mbuf[...]
        for u in range(UNROLL):
            mem = step(i * UNROLL + u, mem)
        mbuf[...] = mem
    _loop(NSEG // UNROLL, steps)

    pltpu.make_async_copy(outbuf, outbuf, sem_out).wait()


@functools.partial(jax.jit, static_argnames=["A_seg_len"])
def pallas_parallel_sum__memory_aug_recurrent_mem_tr__dense_activation_gelu__prompt_kernel(
        A_x, A_mem0, A_Wq, A_Wk, A_Wv, A_Wo, A_seg_len, B_x, B_w1, B_b1, B_w2, B_b2):
    del B_x
    assert A_seg_len == SEG and A_x.shape == (1, S, D) and A_mem0.shape == (1, M, D)
    hbm = pl.BlockSpec(memory_space=pl.ANY)
    dma = pltpu.SemaphoreType.DMA
    out = pl.pallas_call(
        _kernel,
        out_shape=jax.ShapeDtypeStruct((S, D), bf16),
        in_specs=[hbm] * 10,
        out_specs=hbm,
        scratch_shapes=[
            pltpu.VMEM((S, D), bf16),
            pltpu.VMEM((S, D), f32),
            pltpu.VMEM((S, D), f32),
            pltpu.VMEM((S, D), bf16),
            pltpu.VMEM((NPAIR, D, 128), u32),
            pltpu.VMEM((3 * H, D // 2, 128), u32),
            pltpu.VMEM((KT, H * DH // 2, 128), u32),
            pltpu.VMEM((FT, D // 2, 128), u32),
            pltpu.VMEM((KT, F // 2, 128), u32),
            pltpu.VMEM((F,), bf16),
            pltpu.VMEM((D,), bf16),
            pltpu.VMEM((FT, 8, 128), f32),
            pltpu.VMEM((KT, 8, 128), f32),
            pltpu.VMEM((M, D), bf16),
            pltpu.VMEM((M, D), f32),
            pltpu.VMEM((2 * RB, FA * 128), f32),
            dma((3,)), dma((NRB,)), dma((FA,)), dma(()), dma((NPAIR // 8,)), dma(()), dma(()),
        ],
        compiler_params=pltpu.CompilerParams(vmem_limit_bytes=120 * 2**20),
        name="rmt_ffn",
    )(A_x.reshape(S, D), A_mem0.reshape(M, D), A_Wq, A_Wk, A_Wv, A_Wo.reshape(H * DH, D),
      B_w1, B_b1, B_w2, B_b2)
    return out.reshape(1, S, D)
```

```python
import functools

import jax
import jax.numpy as jnp
from jax.experimental import pallas as pl
from jax.experimental.pallas import tpu as pltpu

f32, bf16, u32 = jnp.float32, jnp.bfloat16, jnp.uint32

S, D, H, DH, M, SEG, F = 2048, 1024, 32, 128, 8, 32, 3584
L = M + SEG
NSEG = S // SEG
KT = D // 128
FT = F // 128
FA = 14
RB = 256
NRB = S // RB
HG = 4
G = H // HG
NPAIR = 3 * H // 2
UNROLL = 2


def _gelu(x):
    c = 0.7978845608028654
    hx = 0.5 * x
    return hx + hx * jnp.tanh(x * (c + (c * 0.044715) * (x * x)))


def _mult(v, k):
    return v if isinstance(v, int) else pl.multiple_of(v, k)


def _wt(ref, idxs, rows=None):
    ts = [pltpu.bitcast(ref[i] if rows is None else ref[i, rows, :], bf16) for i in idxs]
    return ts[0] if len(ts) == 1 else jnp.concatenate(ts, axis=1)


def _add_rows(a, b8):
    r, n = a.shape
    return (a.reshape(r // 8, 8, n) + b8[None]).reshape(r, n)


def _loop(n, fn):
    def body(i, carry):
        fn(i)
        return carry
    jax.lax.fori_loop(0, n, body, 0)


def _kernel(x_hbm, mem_hbm, wq_hbm, wk_hbm, wv_hbm, wo_hbm, w1_hbm, b1_hbm, w2_hbm, b2_hbm,
            out_hbm,
            xbuf, xn, acc, outbuf, stage, wqkv, wo, w1, w2, b1v, b2v, b1f, b2f, membuf, mbuf, hbuf,
            sem_small, sem_x, sem_w1a, sem_w2a, sem_st, sem_late, sem_out):
    def cp_x(i):
        rows = pl.ds(_mult(i * RB, RB), RB)
        return pltpu.make_async_copy(x_hbm.at[rows], xbuf.at[rows], sem_x.at[i])

    def cp_w1(t, sem):
        cols = pl.ds(_mult(t * 128, 128), 128)
        return pltpu.make_async_copy(w1_hbm.bitcast(u32).at[:, cols], w1.at[t], sem)

    def cp_w2(c, first, sem):
        rows = pl.ds(0, FA * 64) if first else pl.ds(FA * 64, (FT - FA) * 64)
        cols = pl.ds(_mult(c * 128, 128), 128)
        return pltpu.make_async_copy(w2_hbm.bitcast(u32).at[rows, cols], w2.at[c, rows], sem)

    def cp_wo(c, sem):
        return pltpu.make_async_copy(wo_hbm.bitcast(u32).at[:, pl.ds(c * 128, 128)], wo.at[c], sem)

    def cp_pair(mi, p):
        u = mi * (H // 2) + p
        src = (wq_hbm, wk_hbm, wv_hbm)[mi].bitcast(u32).at[:, p, :]
        return pltpu.make_async_copy(src, stage.at[u], sem_st.at[u // 8])

    def cp_out(r0):
        rows = pl.ds(r0, SEG)
        return pltpu.make_async_copy(outbuf.at[rows], out_hbm.at[rows], sem_out)

    cp_small = (pltpu.make_async_copy(b1_hbm, b1v, sem_small.at[0]),
                pltpu.make_async_copy(b2_hbm, b2v, sem_small.at[1]),
                pltpu.make_async_copy(mem_hbm, membuf, sem_small.at[2]))

    def ln_rows(r0, n):
        xb = xbuf[pl.ds(r0, n), :].astype(f32)
        d = xb - jnp.mean(xb, axis=-1, keepdims=True)
        var = jnp.mean(d * d, axis=-1, keepdims=True)
        xn[pl.ds(r0, n), :] = d * jax.lax.rsqrt(var + 1e-5)

    def up_dot(r0, hr0, t):
        u = jnp.dot(xn[pl.ds(r0, RB), :], _wt(w1, (t, t + 1)), preferred_element_type=f32)
        u = _add_rows(u, jnp.concatenate([b1f[t], b1f[t + 1]], axis=1))
        hbuf[pl.ds(hr0, RB), pl.ds(_mult(t * 128, 128), 256)] = _gelu(u)

    def dn_dot(r0, hr0, c, tie=None):
        r = jnp.dot(hbuf[pl.ds(hr0, RB), :], _wt(w2, (c,), pl.ds(0, FA * 64)), preferred_element_type=f32)
        cs = pl.ds(_mult(c * 128, 128), 128)
        bias = b2f[c] if tie is None else tie(b2f[c])
        acc[pl.ds(r0, RB), cs] = r + _add_rows(xbuf[pl.ds(r0, RB), cs].astype(f32), bias)

    def repack(u, d0, nd):
        a = stage[u, pl.ds(d0, nd), :]
        rows = pl.ds(d0 // 2, nd // 2)
        wqkv[2 * u, rows, :] = pltpu.bitcast(a.astype(jnp.uint16), u32)
        wqkv[2 * u + 1, rows, :] = pltpu.bitcast((a >> 16).astype(jnp.uint16), u32)

    cp_x(0).start()
    cp_x(1).start()
    for c in cp_small:
        c.start()
    _loop(FA, lambda t: cp_w1(t, sem_w1a.at[t]).start())
    _loop(KT, lambda c: cp_w2(c, True, sem_w2a).start())
    for i in range(2, NRB):
        cp_x(i).start()

    cp_x(0).wait()
    for p in range(H // 2):
        cp_pair(0, p).start()
    ln_rows(0, RB)
    cp_x(1).wait()
    ln_rows(RB, RB)
    cp_small[0].wait()
    for t in range(FT):
        b1f[t] = jnp.broadcast_to(b1v[pl.ds(t * 128, 128)].astype(f32)[None, :], (8, 128))

    for t0, t1 in ((0, 2), (2, 6), (6, FA)):
        for t in range(t0, t1):
            cp_w1(t, sem_w1a.at[t]).wait()
        for t in range(t0, t1, 2):
            up_dot(0, 0, t)
            up_dot(RB, RB, t)

    for c in range(KT):
        cp_w2(c, True, sem_w2a).wait()
    cp_x(2).wait()
    cp_small[1].wait()
    cp_small[2].wait()
    mbuf[...] = membuf[...].astype(f32)
    for c in range(KT):
        b2f[c] = jnp.broadcast_to(b2v[pl.ds(c * 128, 128)].astype(f32)[None, :], (8, 128))
    for mi in (1, 2):
        for p in range(H // 2):
            cp_pair(mi, p).start()

    def dn_first(i):
        n = RB // 4
        for k in range(2):
            c = 2 * (2 * i + k)
            dn_dot(0, 0, c)
            dn_dot(RB, RB, c)
            ln_rows(pl.multiple_of(2 * RB + (2 * i + k) * n, n), n)
            dn_dot(0, 0, c + 1)
            dn_dot(RB, RB, c + 1)
    _loop(2, dn_first)

    for i in range(3, NRB):
        cp_x(i).wait()
    ndot = FA // 2 + KT
    pieces = [(u, d0) for u in range(8) for d0 in range(0, D, 128)]

    def ffn_block(j):
        r0 = pl.multiple_of((j + 2) * RB, RB)
        rn = pl.multiple_of(jnp.minimum(j + 3, NRB - 1) * RB, RB)
        chunk = stage.at[pl.ds(j * 8, 8)]
        pltpu.make_async_copy(chunk, chunk, sem_st.at[j]).wait()

        @pl.when(j == 1)
        def _():
            for c in range(KT):
                cp_wo(c, sem_late).start()
            for t in range(FA, FT):
                cp_w1(t, sem_late).start()
            for c in range(KT):
                cp_w2(c, False, sem_late).start()

        def repack_part(i):
            for u, d0 in pieces[i * len(pieces) // (ndot - 1):(i + 1) * len(pieces) // (ndot - 1)]:
                repack(j * 8 + u, d0, 128)

        for i, t in enumerate(range(0, FA, 2)):
            if i >= 1:
                repack_part(i - 1)
            up_dot(r0, 0, t)
        live = j < NRB
        n = RB // KT
        for c in range(KT):
            repack_part(FA // 2 + c - 1)
            for r in range(0, n, 8):
                ln_rows(pl.multiple_of(rn + c * n + r, 8), 8)
            done = xn[pl.ds(pl.multiple_of(rn + (c + 1) * n - 8, 8), 8), 0:128]
            dn_dot(r0, 0, c, lambda b, done=done: jnp.where(live, b, done))
    _loop(NRB - 2, ffn_block)

    for c in range(KT):
        cp_wo(c, sem_late).wait()
    for t in range(FA, FT):
        cp_w1(t, sem_late).wait()
    for c in range(KT):
        cp_w2(c, False, sem_late).wait()

    scale = DH ** -0.5

    def step(s, mem):
        ii = jax.lax.broadcasted_iota(jnp.int32, (L, L), 0)
        jj = jax.lax.broadcasted_iota(jnp.int32, (L, L), 1)
        mask = (ii < M) | (ii >= jj)
        r0 = pl.multiple_of(s * SEG, SEG)
        xs = xn[pl.ds(r0, SEG), :]
        h = jnp.concatenate([mem, xs], axis=0)
        q, k, v, e, rl, o, ff = {}, {}, {}, {}, {}, {}, {}
        st = dict(attn=None, ffn=None)
        heads = lambda g, mi: range(mi * H + g * HG, mi * H + (g + 1) * HG)
        lanes = [slice(j * DH, (j + 1) * DH) for j in range(HG)]

        def proj(dst, g, mi):
            dst[g] = jnp.dot(h, _wt(wqkv, heads(g, mi)), preferred_element_type=f32)

        def scores(g):
            e[g], rl[g] = [], []
            for sl in lanes:
                sc = jax.lax.dot_general(q[g][:, sl], k[g][:, sl].astype(bf16), (((1,), (1,)), ((), ())),
                                         preferred_element_type=f32) * scale
                sc = jnp.where(mask, sc, -1e9)
                ex = jnp.exp(sc - jnp.max(sc, axis=-1, keepdims=True))
                tot = jnp.sum(ex, axis=-1, keepdims=True)
                r = pltpu.reciprocal(tot, approx=True)
                e[g].append(ex)
                rl[g].append(r * (2.0 - tot * r))

        def pv(g):
            o[g] = jnp.concatenate(
                [jnp.dot(e[g][j], v[g][:, sl].astype(bf16), preferred_element_type=f32) * rl[g][j]
                 for j, sl in enumerate(lanes)], axis=1)

        def out_proj(g):
            r = jnp.dot(o[g], _wt(wo, range(KT), pl.ds(g * HG * 64, HG * 64)), preferred_element_type=f32)
            st["attn"] = r if st["attn"] is None else st["attn"] + r

        def up(i, t0, t1):
            u = jnp.dot(xs, _wt(w1, range(t0, t1)), preferred_element_type=f32)
            ff[i] = _gelu(_add_rows(u, jnp.concatenate([b1f[t] for t in range(t0, t1)], axis=1)))

        def down(i, t0, t1):
            r = jnp.dot(ff[i], _wt(w2, range(KT), pl.ds(t0 * 64, (t1 - t0) * 64)), preferred_element_type=f32)
            st["ffn"] = (acc[pl.ds(r0, SEG), :] if st["ffn"] is None else st["ffn"]) + r

        mid = FA + 8
        proj(q, 0, 0)
        proj(k, 0, 1)
        proj(v, 0, 2)
        for g in range(G):
            last = g + 1 == G
            up(0, FA, mid) if last else proj(q, g + 1, 0)
            scores(g)
            up(1, mid, FT) if last else proj(k, g + 1, 1)
            if g == 0:
                proj(v, 1, 2)
            else:
                out_proj(g - 1)
            pv(g)
            if 0 < g < G - 1:
                proj(v, g + 1, 2)
        down(0, FA, mid)
        out_proj(G - 1)
        attn = st["attn"]
        down(1, mid, FT)
        outbuf[pl.ds(r0, SEG), :] = (attn[M:L] + st["ffn"]).astype(bf16)
        cp_out(r0).start()
        return attn[0:M]

    def steps(i):
        mem = mbuf[...]
        for u in range(UNROLL):
            mem = step(i * UNROLL + u, mem)
        mbuf[...] = mem
    _loop(NSEG // UNROLL, steps)

    pltpu.make_async_copy(outbuf, outbuf, sem_out).wait()


@functools.partial(jax.jit, static_argnames=["A_seg_len"])
def pallas_parallel_sum__memory_aug_recurrent_mem_tr__dense_activation_gelu__prompt_kernel(
        A_x, A_mem0, A_Wq, A_Wk, A_Wv, A_Wo, A_seg_len, B_x, B_w1, B_b1, B_w2, B_b2):
    del B_x
    assert A_seg_len == SEG and A_x.shape == (1, S, D) and A_mem0.shape == (1, M, D)
    hbm = pl.BlockSpec(memory_space=pl.ANY)
    dma = pltpu.SemaphoreType.DMA
    out = pl.pallas_call(
        _kernel,
        out_shape=jax.ShapeDtypeStruct((S, D), bf16),
        in_specs=[hbm] * 10,
        out_specs=hbm,
        scratch_shapes=[
            pltpu.VMEM((S, D), bf16),
            pltpu.VMEM((S, D), f32),
            pltpu.VMEM((S, D), f32),
            pltpu.VMEM((S, D), bf16),
            pltpu.VMEM((NPAIR, D, 128), u32),
            pltpu.VMEM((3 * H, D // 2, 128), u32),
            pltpu.VMEM((KT, H * DH // 2, 128), u32),
            pltpu.VMEM((FT, D // 2, 128), u32),
            pltpu.VMEM((KT, F // 2, 128), u32),
            pltpu.VMEM((F,), bf16),
            pltpu.VMEM((D,), bf16),
            pltpu.VMEM((FT, 8, 128), f32),
            pltpu.VMEM((KT, 8, 128), f32),
            pltpu.VMEM((M, D), bf16),
            pltpu.VMEM((M, D), f32),
            pltpu.VMEM((2 * RB, FA * 128), f32),
            dma((3,)), dma((NRB,)), dma((FA,)), dma(()), dma((NPAIR // 8,)), dma(()), dma(()),
        ],
        compiler_params=pltpu.CompilerParams(vmem_limit_bytes=120 * 2**20),
        name="rmt_ffn",
    )(A_x.reshape(S, D), A_mem0.reshape(M, D), A_Wq, A_Wk, A_Wv, A_Wo.reshape(H * DH, D),
      B_w1, B_b1, B_w2, B_b2)
    return out.reshape(1, S, D)
```
